```python
import os as _os
_os.environ.setdefault("JAX_PLATFORMS", "cpu")
import jax
import jax.numpy as jnp

def _softmax(x, axis=-1):
    return jax.nn.softmax(x, axis=axis)
def _gelu(x):
    return jax.nn.gelu(x, approximate=True)
def _silu(x):
    return jax.nn.silu(x)
def _sigmoid(x):
    return jax.nn.sigmoid(x)
def _layernorm(x, axis=-1, eps=1e-5):
    m = jnp.mean(x, axis=axis, keepdims=True)
    v = jnp.var(x, axis=axis, keepdims=True)
    return (x - m) / jnp.sqrt(v + eps)
def _scatter_add(tgt, idx, src, axis=0):
    return tgt.at[idx].add(src)
def _segment_sum(src, seg, n):
    return jax.ops.segment_sum(src, seg, n)
class _Rng:
    def __init__(self, key):
        self._k = key
    def _next(self):
        self._k, sub = jax.random.split(self._k)
        return sub
    def normal(self, shape):
        return jax.random.normal(self._next(), shape, dtype=jnp.bfloat16)
    def randint(self, lo, hi, shape):
        return jax.random.randint(self._next(), shape, lo, hi, dtype=jnp.int32)
    def uniform(self, shape, lo=0.0, hi=1.0):
        return jax.random.uniform(self._next(), shape, jnp.bfloat16, lo, hi)
    def permutation(self, n):
        return jax.random.permutation(self._next(), n)


kernel_name = 'standalone__mha_block_cached__near_ridge'

def setup_inputs():
    _rng = _Rng(jax.random.key(int.from_bytes(__import__("os").urandom(4), "little")))
    _w = (lambda a: (lambda t: t.astype(jnp.bfloat16) if jnp.issubdtype(t.dtype, jnp.floating) else t)(jnp.asarray(a)))
    B, Sq, D = 8, 96, 576
    H, Sk, Dh = 32, 96, 128
    return {
        "x": _w((lambda *s: _rng.normal(s) * 0.8)(B, Sq, D)),
        "k_cache": _w((lambda *s: _rng.normal(s) * 0.8)(B, H, Sk, Dh)),
        "v_cache": _w((lambda *s: _rng.normal(s) * 0.05)(B, H, Sk, Dh)),
        "wq": _w((lambda *s: _rng.normal(s) * 0.8)(D, H * Dh) * (D ** -0.5)),
        "wo": _w((lambda *s: _rng.normal(s) * 0.05)(H * Dh, D) * ((H * Dh) ** -0.5)),
    }

def reference(x, k_cache, v_cache, wq, wo):
    B, Sq, D = x.shape
    H, Dh = 32, 128
    q = (lambda x, *d: x.transpose(*d))((x @ wq).reshape(B, Sq, H, Dh), 0, 2, 1, 3)
    scores = jnp.einsum("bhqd,bhkd->bhqk", q, k_cache) * (Dh ** -0.5)
    p = _softmax(scores, axis=-1)
    o = jnp.einsum("bhqk,bhkd->bhqd", p, v_cache)
    return (lambda x, *d: x.transpose(*d))(o, 0, 2, 1, 3).reshape(B, Sq, H * Dh) @ wo
```

```python
import math

import jax
import jax.numpy as jnp
import jax.experimental.pallas as pl
import jax.experimental.pallas.tpu as pltpu

HG = 4
STAGES = ((128, 1), (192, 2), (256, 3), (384, 4), (640, 5), (640, 13), (768, 16))
BARS = (36, 58)
FIRST = 36
BURST = 4
ENDCALM = 4


def _build_program(B, NG, NT, M):
    H = NG * HG
    nj = NG * B

    def block(r0, r1, n0, n1):
        out = []
        n = n0
        while n < n1:
            if n % HG == 0 and n + HG <= n1:
                out.append(('AR', r0, r1, n, n + HG))
                out += [('AM', m, r0, r1) for m in range(n, n + HG)]
                n += HG
            elif n % 2 == 0 and n + 2 <= n1:
                h = (r0 + r1) // 2
                out += [('AR', r0, h, n, n + 2), ('AR', h, r1, n, n + 2)]
                out += [('AM', m, r0, r1) for m in range(n, n + 2)]
                n += 2
            else:
                q4 = (r1 - r0) // 4
                out += [('AR', r0 + i * q4, r0 + (i + 1) * q4, n, n + 1) for i in range(4)]
                out.append(('AM', n, r0, r1))
                n += 1
        return out

    prog = []
    px, pw = 0, 0
    for (cx, cw) in STAGES:
        prog.append('W')
        if cw > pw and cx > px and px > 0:
            prog += block(px, cx, 0, pw)
            prog += block(0, cx, pw, cw)
        elif cx > px:
            prog += block(px, cx, 0, cw)
        else:
            prog += block(0, cx, pw, cw)
        px, pw = cx, cw
    assert px == M and pw % HG == 0
    g0 = pw // HG

    def cbig(g, ts):
        return [('CR', g, t) for t in ts]

    bigs = [None] * (5 * g0)
    for g in range(g0, NG):
        bigs += block(0, M, g * HG, (g + 1) * HG)
    for g in range(NG - 3):
        bigs += cbig(g, range(NT))
    bigs += cbig(NG - 3, range(NT - 1)) + cbig(NG - 2, range(NT - 1)) + cbig(NG - 1, range(NT - 3))
    tail = [('CR', NG - 1, NT - 3), ('CR', NG - 1, NT - 2), ('CR', NG - 3, NT - 1), ('PV', nj - 1),
            ('CR', NG - 2, NT - 1), ('CF', NG - 1, NT - 1)]

    ngap = len(bigs) - FIRST
    extra = nj - ngap
    cnt = [1] * ngap
    burst = min(BURST, extra)
    for i in range(burst):
        cnt[i] = 2
    rest = extra - burst
    if rest > 0:
        span = ngap - burst - ENDCALM
        for r in range(rest):
            cnt[burst + int((r + 0.5) * span / rest)] += 1
    assert sum(cnt) == nj

    jn = 0
    prev = []
    for i, bg in enumerate(bigs):
        if bg is not None:
            prog.append(bg)
        if (i + 1) in BARS:
            prog.append('W')
        if i >= FIRST:
            cur = list(range(jn, jn + cnt[i - FIRST]))
            jn += cnt[i - FIRST]
            qks = [('QK', j) for j in cur]
            pvs = [('PV', j) for j in prev]
            prog += (pvs + qks) if (i + 1) in BARS else (qks + pvs)
            prev = cur
    assert prev == [nj - 1]
    xsplit = sorted(set([0] + [s[0] for s in STAGES]))
    wsplit = sorted(set([0] + [s[1] for s in STAGES] + list(range(0, H + 1, HG))))
    return prog + tail, xsplit, wsplit


@jax.jit
def pallas_standalone__mha_block_cached__near_ridge_kernel(
    x: jax.Array,
    k_cache: jax.Array,
    v_cache: jax.Array,
    wq: jax.Array,
    wo: jax.Array,
):
    B, Sq, D = x.shape
    _, H, Sk, Dh = k_cache.shape
    M = B * Sq
    x2 = x.reshape(M, D)
    wot = wo.T
    NG = H // HG
    GW = HG * Dh
    c = (Dh ** -0.5) * math.log2(math.e)
    NT = M // 128
    NB = -(-D // 128)
    DM = (D // 128) * 128
    KT = DM // 128
    assert KT == HG and GW // 128 == HG and D > DM

    prog, xsplit, wsplit = _build_program(B, NG, NT, M)

    bmax = [((t + 1) * 128 - 1) // Sq for t in range(NT)]
    seq = [it for it in prog if it != 'W']
    pos = {it: i for i, it in enumerate(seq)}
    assert len(pos) == len(seq)
    for it in seq:
        if it[0] in ('CR', 'CF'):
            assert pos[('PV', it[1] * B + bmax[it[2]])] < pos[it], it
        if it[0] == 'PV':
            assert pos[('QK', it[1])] < pos[it], it
        if it[0] == 'QK':
            assert all(pos[z] < pos[it] for z in seq if z[0] == 'AM' and z[1] // HG == it[1] // B)

    def xneeds(r0, r1):
        return [('x', i) for i in range(len(xsplit) - 1) if xsplit[i] < r1 and xsplit[i + 1] > r0]

    def wneeds(n0, n1):
        return [('wq', i) for i in range(len(wsplit) - 1) if wsplit[i] < n1 and wsplit[i + 1] > n0]

    def needs(it):
        k = it[0]
        if k == 'AR':
            return xneeds(it[1], it[2]) + wneeds(it[3], it[4])
        if k == 'AM':
            return xneeds(it[2], it[3]) + wneeds(it[1], it[1] + 1)
        if k in ('CR', 'CF'):
            return [('wo', it[1])]
        if k == 'QK':
            return [('k', it[1] // B)]
        return [('v', it[1] // B)]

    groups = []
    seen = set()
    for it in prog:
        if it == 'W':
            groups.append([])
            continue
        for n in needs(it):
            if n not in seen:
                seen.add(n)
                groups[-1].append(n)
    sem_id = {n: gi for gi, grp in enumerate(groups) for n in grp}
    outs = [('out', t) for t in range(NT - 1)] + [('outc', n) for n in range(NB)]
    for o_ in outs:
        sem_id[o_] = len(groups)
    nsem = len(groups) + 1
    cr_first, cr_last = {}, {}
    for it in seq:
        if it[0] == 'CR':
            cr_first.setdefault(it[2], it[1])
            cr_last[it[2]] = it[1]

    nt_dims = (((1,), (1,)), ((), ()))

    def kernel(x_hbm, k_hbm, v_hbm, wq_hbm, wot_hbm, out_hbm,
               x_v, wq_v, k_v, v_v, wot_v, q_s, qp, o_s, acc, accl, sems):
        out_v = o_s.at[NG]

        def cp(name):
            kind, g = name
            s = sems.at[sem_id[name]]
            if kind == 'x':
                r0, r1 = xsplit[g], xsplit[g + 1]
                return pltpu.make_async_copy(x_hbm.at[pl.ds(r0, r1 - r0)], x_v.at[pl.ds(r0, r1 - r0)], s)
            if kind == 'wq':
                n0, n1 = wsplit[g], wsplit[g + 1]
                return pltpu.make_async_copy(wq_hbm.at[:, pl.ds(n0 * Dh, (n1 - n0) * Dh)],
                                             wq_v.at[n0 // HG, :, pl.ds((n0 % HG) * Dh, (n1 - n0) * Dh)], s)
            if kind == 'k':
                return pltpu.make_async_copy(k_hbm.at[:, pl.ds(g * HG, HG)], k_v.at[g], s)
            if kind == 'v':
                return pltpu.make_async_copy(v_hbm.at[:, pl.ds(g * HG, HG)], v_v.at[g], s)
            if kind == 'wo':
                return pltpu.make_async_copy(wot_hbm.at[:, pl.ds(g * GW, GW)], wot_v.at[g], s)
            if kind == 'out':
                return pltpu.make_async_copy(out_v.at[pl.ds(g * 128, 128)], out_hbm.at[pl.ds(g * 128, 128)], s)
            w = min(128, D - g * 128)
            return pltpu.make_async_copy(out_v.at[pl.ds(M - 128, 128), pl.ds(g * 128, w)],
                                         out_hbm.at[pl.ds(M - 128, 128), pl.ds(g * 128, w)], s)

        def AR(r0, r1, n0, n1):
            g, a, b_ = n0 // HG, (n0 % HG) * Dh, ((n1 - 1) % HG + 1) * Dh
            qp[g % 2, r0:r1, a:b_] = jnp.dot(x_v[r0:r1, DM:], wq_v[g, DM:, a:b_],
                                             preferred_element_type=jnp.float32)

        def AM(n, r0, r1):
            g, a = n // HG, (n % HG) * Dh
            ds = [jnp.dot(x_v[r0:r1, kt * 128:(kt + 1) * 128], wq_v[g, kt * 128:(kt + 1) * 128, a:a + Dh],
                          preferred_element_type=jnp.float32) for kt in range(KT)]
            d = (ds[0] + ds[1]) + ((ds[2] + ds[3]) + qp[g % 2, r0:r1, a:a + Dh])
            q_s[g, r0:r1, a:a + Dh] = d.astype(jnp.bfloat16)

        def CR(g, t):
            ds = [jax.lax.dot_general(wot_v[g, :, kt * 128:(kt + 1) * 128],
                                      o_s[g, t * 128:(t + 1) * 128, kt * 128:(kt + 1) * 128],
                                      nt_dims, preferred_element_type=jnp.float32) for kt in range(HG)]
            e = ds[2] + ds[3]
            if g != cr_first[t]:
                e = e + acc[:, t * 128:(t + 1) * 128]
            d = (ds[0] + ds[1]) + e
            if g == cr_last[t] and t == NT - 1:
                accl[...] = d.T
            elif g == cr_last[t]:
                out_v[t * 128:(t + 1) * 128, :] = d.T.astype(jnp.bfloat16)
                cp(('out', t)).start()
            else:
                acc[:, t * 128:(t + 1) * 128] = d

        def CF(g, t):
            o = o_s[g, t * 128:(t + 1) * 128, :GW]
            for n in range(NB):
                w = min(128, D - n * 128)
                d = jax.lax.dot_general(o, wot_v[g, n * 128:n * 128 + w, :], nt_dims,
                                        preferred_element_type=jnp.float32)
                d = d + accl[:, n * 128:n * 128 + w]
                out_v[t * 128:(t + 1) * 128, n * 128:n * 128 + w] = d.astype(jnp.bfloat16)
                cp(('outc', n)).start()

        pend = {}

        def QK(j):
            g, b = divmod(j, B)
            ps = []
            for h in range(HG):
                qh = q_s[g, b * Sq:(b + 1) * Sq, h * Dh:(h + 1) * Dh]
                s = jax.lax.dot_general(qh, k_v[g, b, h], nt_dims, preferred_element_type=jnp.float32)
                m = jnp.max(s, axis=-1, keepdims=True)
                p = jnp.exp2((s - m) * c)
                l = jnp.sum(p, axis=-1, keepdims=True)
                r = pl.reciprocal(l, approx=True)
                r = r * (2.0 - l * r)
                ps.append((p * r).astype(jnp.bfloat16))
            pend[j] = ps

        def PV(j):
            g, b = divmod(j, B)
            ps = pend.pop(j)
            for h in range(HG):
                o = jnp.dot(ps[h], v_v[g, b, h], preferred_element_type=jnp.float32)
                o_s[g, b * Sq:(b + 1) * Sq, h * Dh:(h + 1) * Dh] = o.astype(jnp.bfloat16)

        rounds = {'AR': AR, 'AM': AM, 'CR': CR, 'CF': CF, 'QK': QK, 'PV': PV}

        for grp in groups:
            for n in grp:
                cp(n).start()
        gi = 0
        for it in prog:
            if it == 'W':
                for n in groups[gi]:
                    cp(n).wait()
                gi += 1
            else:
                rounds[it[0]](*it[1:])
        for o_ in outs:
            cp(o_).wait()

    out = pl.pallas_call(
        kernel,
        in_specs=[pl.BlockSpec(memory_space=pl.ANY)] * 5,
        out_specs=pl.BlockSpec(memory_space=pl.ANY),
        out_shape=jax.ShapeDtypeStruct((M, D), x.dtype),
        scratch_shapes=[
            pltpu.VMEM((M, D), jnp.bfloat16),
            pltpu.VMEM((NG, D, GW), jnp.bfloat16),
            pltpu.VMEM((NG, B, HG, Sk, Dh), jnp.bfloat16),
            pltpu.VMEM((NG, B, HG, Sk, Dh), jnp.bfloat16),
            pltpu.VMEM((NG, D, GW), jnp.bfloat16),
            pltpu.VMEM((NG, M, GW), jnp.bfloat16),
            pltpu.VMEM((2, M, GW), jnp.float32),
            pltpu.VMEM((NG + 1, M, D), jnp.bfloat16),
            pltpu.VMEM((D, M), jnp.float32),
            pltpu.VMEM((128, D), jnp.float32),
            pltpu.SemaphoreType.DMA((nsem,)),
        ],
        compiler_params=pltpu.CompilerParams(
            vmem_limit_bytes=100 * 1024 * 1024,
        ),
    )(x2, k_cache, v_cache, wq, wot)
    return out.reshape(B, Sq, D)
```

```python
import math

import jax
import jax.numpy as jnp
import jax.experimental.pallas as pl
import jax.experimental.pallas.tpu as pltpu

HG = 4
STAGES = ((256, 1), (576, 2), (768, 8))
BARS = (0, 12, 32, 50)
FIRST = 23
DOUBLE0 = 32
ENDCALM = 4


def _build_program(B, NG, NT, M):
    nj = NG * B

    prog = []
    px, pw = 0, 0
    for (cx, cw) in STAGES:
        prog.append('W')
        if cx > px:
            prog += [('AR', g, px, cx) for g in range(pw)]
        prog += [('AR', g, 0, cx) for g in range(pw, cw)]
        px, pw = cx, cw
    assert px == M and pw == NG

    def cbig(g, ts):
        return [('CR', g, t) for t in ts]

    bigs = [('AM', n) for n in range(NG * HG)]
    for g in range(NG - 3):
        bigs += cbig(g, range(NT))
    bigs += cbig(NG - 3, range(NT - 1)) + cbig(NG - 2, range(NT - 1)) + cbig(NG - 1, range(NT - 3))
    tail = [('CR', NG - 1, NT - 3), ('CR', NG - 1, NT - 2), ('CR', NG - 3, NT - 1), ('PV', nj - 1),
            ('CR', NG - 2, NT - 1), ('CF', NG - 1, NT - 1)]

    ngap = len(bigs) - FIRST
    extra = nj - ngap
    cnt = [1] * ngap
    lo = DOUBLE0 - FIRST
    span = ngap - lo - ENDCALM
    for r in range(extra):
        cnt[lo + int((r + 0.5) * span / extra)] += 1
    assert sum(cnt) == nj

    jn = 0
    prev = []
    if 0 in BARS:
        prog.append('W')
    for i, bg in enumerate(bigs):
        prog.append(bg)
        if (i + 1) in BARS:
            prog.append('W')
        if i >= FIRST:
            cur = list(range(jn, jn + cnt[i - FIRST]))
            jn += cnt[i - FIRST]
            qks = [('QK', j) for j in cur]
            pvs = [('PV', j) for j in prev]
            prog += (pvs + qks) if (i + 1) in BARS else (qks + pvs)
            prev = cur
    assert prev == [nj - 1]
    xsplit = sorted(set([0] + [s[0] for s in STAGES]))
    wsplit = sorted(set([0] + [s[1] for s in STAGES]))
    return prog + tail, xsplit, wsplit


@jax.jit
def pallas_standalone__mha_block_cached__near_ridge_kernel(
    x: jax.Array,
    k_cache: jax.Array,
    v_cache: jax.Array,
    wq: jax.Array,
    wo: jax.Array,
):
    B, Sq, D = x.shape
    _, H, Sk, Dh = k_cache.shape
    M = B * Sq
    x2 = x.reshape(M, D)
    wot = wo.T
    NG = H // HG
    GW = HG * Dh
    c = (Dh ** -0.5) * math.log2(math.e)
    NT = M // 128
    NB = -(-D // 128)
    DM = (D // 128) * 128
    DR = D - DM
    KT = DM // 128
    assert KT == HG and GW // 128 == HG and DR > 0

    prog, xsplit, wsplit = _build_program(B, NG, NT, M)

    bmax = [((t + 1) * 128 - 1) // Sq for t in range(NT)]
    seq = [it for it in prog if it != 'W']
    pos = {it: i for i, it in enumerate(seq)}
    assert len(pos) == len(seq)
    for it in seq:
        if it[0] in ('CR', 'CF'):
            assert pos[('PV', it[1] * B + bmax[it[2]])] < pos[it], it
        if it[0] == 'PV':
            assert pos[('QK', it[1])] < pos[it], it
        if it[0] == 'QK':
            assert all(pos[z] < pos[it] for z in seq if z[0] == 'AM' and z[1] // HG == it[1] // B)

    def needs(it):
        k = it[0]
        if k == 'AR':
            g, r0, r1 = it[1:]
            return ([('xr', i) for i in range(len(xsplit) - 1) if xsplit[i] < r1 and xsplit[i + 1] > r0]
                    + [('wr', i) for i in range(len(wsplit) - 1) if wsplit[i] <= g < wsplit[i + 1]])
        if k == 'AM':
            return [('xm', 0), ('wq', it[1] // HG)]
        if k in ('CR', 'CF'):
            return [('wo', it[1])]
        if k == 'QK':
            return [('k', it[1] // B)]
        return [('v', it[1] // B)]

    groups = []
    seen = set()
    for it in prog:
        if it == 'W':
            groups.append([])
            continue
        for n in needs(it):
            if n not in seen:
                seen.add(n)
                groups[-1].append(n)
    sem_id = {n: gi for gi, grp in enumerate(groups) for n in grp}
    outs = [('out', t) for t in range(NT - 1)] + [('outc', n) for n in range(NB)]
    for o_ in outs:
        sem_id[o_] = len(groups)
    nsem = len(groups) + 1
    cr_first, cr_last = {}, {}
    for it in seq:
        if it[0] == 'CR':
            cr_first.setdefault(it[2], it[1])
            cr_last[it[2]] = it[1]

    nt_dims = (((1,), (1,)), ((), ()))

    def kernel(x_hbm, k_hbm, v_hbm, wq_hbm, wot_hbm, out_hbm,
               x_v, wq_v, wr_v, k_v, v_v, wot_v, q_s, qp, o_s, acc, accl, sems):
        out_v = o_s.at[NG]

        def cp(name):
            kind, g = name
            s = sems.at[sem_id[name]]
            if kind == 'xr':
                r0, r1 = xsplit[g], xsplit[g + 1]
                return pltpu.make_async_copy(x_hbm.at[pl.ds(r0, r1 - r0), pl.ds(DM, DR)],
                                             x_v.at[pl.ds(r0, r1 - r0), pl.ds(DM, DR)], s)
            if kind == 'xm':
                return pltpu.make_async_copy(x_hbm.at[:, pl.ds(0, DM)], x_v.at[:, pl.ds(0, DM)], s)
            if kind == 'wr':
                c0, c1 = wsplit[g] * GW, wsplit[g + 1] * GW
                return pltpu.make_async_copy(wq_hbm.at[pl.ds(DM, DR), pl.ds(c0, c1 - c0)],
                                             wr_v.at[:, pl.ds(c0, c1 - c0)], s)
            if kind == 'wq':
                return pltpu.make_async_copy(wq_hbm.at[pl.ds(0, DM), pl.ds(g * GW, GW)], wq_v.at[g], s)
            if kind == 'k':
                return pltpu.make_async_copy(k_hbm.at[:, pl.ds(g * HG, HG)], k_v.at[g], s)
            if kind == 'v':
                return pltpu.make_async_copy(v_hbm.at[:, pl.ds(g * HG, HG)], v_v.at[g], s)
            if kind == 'wo':
                return pltpu.make_async_copy(wot_hbm.at[:, pl.ds(g * GW, GW)], wot_v.at[g], s)
            if kind == 'out':
                return pltpu.make_async_copy(out_v.at[pl.ds(g * 128, 128)], out_hbm.at[pl.ds(g * 128, 128)], s)
            w = min(128, D - g * 128)
            return pltpu.make_async_copy(out_v.at[pl.ds(M - 128, 128), pl.ds(g * 128, w)],
                                         out_hbm.at[pl.ds(M - 128, 128), pl.ds(g * 128, w)], s)

        def AR(g, r0, r1):
            qp[g, r0:r1, :] = jnp.dot(x_v[r0:r1, DM:], wr_v[:, g * GW:(g + 1) * GW],
                                      preferred_element_type=jnp.float32)

        def AM(n):
            g, a = n // HG, (n % HG) * Dh
            ds = [jnp.dot(x_v[:, kt * 128:(kt + 1) * 128], wq_v[g, kt * 128:(kt + 1) * 128, a:a + Dh],
                          preferred_element_type=jnp.float32) for kt in range(KT)]
            d = (ds[0] + ds[1]) + ((ds[2] + ds[3]) + qp[g, :, a:a + Dh])
            q_s[g, :, a:a + Dh] = d.astype(jnp.bfloat16)

        def CR(g, t):
            ds = [jax.lax.dot_general(wot_v[g, :, kt * 128:(kt + 1) * 128],
                                      o_s[g, t * 128:(t + 1) * 128, kt * 128:(kt + 1) * 128],
                                      nt_dims, preferred_element_type=jnp.float32) for kt in range(HG)]
            e = ds[2] + ds[3]
            if g != cr_first[t]:
                e = e + acc[:, t * 128:(t + 1) * 128]
            d = (ds[0] + ds[1]) + e
            if g == cr_last[t] and t == NT - 1:
                accl[...] = d.T
            elif g == cr_last[t]:
                out_v[t * 128:(t + 1) * 128, :] = d.T.astype(jnp.bfloat16)
                cp(('out', t)).start()
            else:
                acc[:, t * 128:(t + 1) * 128] = d

        def CF(g, t):
            o = o_s[g, t * 128:(t + 1) * 128, :GW]
            for n in range(NB):
                w = min(128, D - n * 128)
                d = jax.lax.dot_general(o, wot_v[g, n * 128:n * 128 + w, :], nt_dims,
                                        preferred_element_type=jnp.float32)
                d = d + accl[:, n * 128:n * 128 + w]
                out_v[t * 128:(t + 1) * 128, n * 128:n * 128 + w] = d.astype(jnp.bfloat16)
                cp(('outc', n)).start()

        pend = {}

        def QK(j):
            g, b = divmod(j, B)
            ps = []
            for h in range(HG):
                qh = q_s[g, b * Sq:(b + 1) * Sq, h * Dh:(h + 1) * Dh]
                s = jax.lax.dot_general(qh, k_v[g, b, h], nt_dims, preferred_element_type=jnp.float32)
                m = jnp.max(s, axis=-1, keepdims=True)
                p = jnp.exp2((s - m) * c)
                l = jnp.sum(p, axis=-1, keepdims=True)
                r = pl.reciprocal(l, approx=True)
                r = r * (2.0 - l * r)
                ps.append((p * r).astype(jnp.bfloat16))
            pend[j] = ps

        def PV(j):
            g, b = divmod(j, B)
            ps = pend.pop(j)
            for h in range(HG):
                o = jnp.dot(ps[h], v_v[g, b, h], preferred_element_type=jnp.float32)
                o_s[g, b * Sq:(b + 1) * Sq, h * Dh:(h + 1) * Dh] = o.astype(jnp.bfloat16)

        rounds = {'AR': AR, 'AM': AM, 'CR': CR, 'CF': CF, 'QK': QK, 'PV': PV}

        for grp in groups:
            for n in grp:
                cp(n).start()
        gi = 0
        for it in prog:
            if it == 'W':
                for n in groups[gi]:
                    cp(n).wait()
                gi += 1
            else:
                rounds[it[0]](*it[1:])
        for o_ in outs:
            cp(o_).wait()

    out = pl.pallas_call(
        kernel,
        in_specs=[pl.BlockSpec(memory_space=pl.ANY)] * 5,
        out_specs=pl.BlockSpec(memory_space=pl.ANY),
        out_shape=jax.ShapeDtypeStruct((M, D), x.dtype),
        scratch_shapes=[
            pltpu.VMEM((M, D), jnp.bfloat16),
            pltpu.VMEM((NG, DM, GW), jnp.bfloat16),
            pltpu.VMEM((DR, H * Dh), jnp.bfloat16),
            pltpu.VMEM((NG, B, HG, Sk, Dh), jnp.bfloat16),
            pltpu.VMEM((NG, B, HG, Sk, Dh), jnp.bfloat16),
            pltpu.VMEM((NG, D, GW), jnp.bfloat16),
            pltpu.VMEM((NG, M, GW), jnp.bfloat16),
            pltpu.VMEM((NG, M, GW), jnp.float32),
            pltpu.VMEM((NG + 1, M, D), jnp.bfloat16),
            pltpu.VMEM((D, M), jnp.float32),
            pltpu.VMEM((128, D), jnp.float32),
            pltpu.SemaphoreType.DMA((nsem,)),
        ],
        compiler_params=pltpu.CompilerParams(
            vmem_limit_bytes=110 * 1024 * 1024,
        ),
    )(x2, k_cache, v_cache, wq, wot)
    return out.reshape(B, Sq, D)
```
